```python
import jax
import jax.numpy as jnp

def _softmax(x, axis=-1):
    return jax.nn.softmax(x, axis=axis)
def _gelu(x):
    return jax.nn.gelu(x, approximate=True)
def _silu(x):
    return jax.nn.silu(x)
def _sigmoid(x):
    return jax.nn.sigmoid(x)
def _layernorm(x, axis=-1, eps=1e-5):
    m = jnp.mean(x, axis=axis, keepdims=True)
    v = jnp.var(x, axis=axis, keepdims=True)
    return (x - m) / jnp.sqrt(v + eps)
def _scatter_add(tgt, idx, src, axis=0):
    return tgt.at[idx].add(src)
def _segment_sum(src, seg, n):
    return jax.ops.segment_sum(src, seg, n)
class _Rng:
    def __init__(self, key):
        self._k = key
    def _next(self):
        self._k, sub = jax.random.split(self._k)
        return sub
    def normal(self, shape):
        return jax.random.normal(self._next(), shape, dtype=jnp.bfloat16)
    def randint(self, lo, hi, shape):
        return jax.random.randint(self._next(), shape, lo, hi, dtype=jnp.int32)
    def uniform(self, shape, lo=0.0, hi=1.0):
        return jax.random.uniform(self._next(), shape, jnp.bfloat16, lo, hi)
    def permutation(self, n):
        return jax.random.permutation(self._next(), n)


kernel_name = 'gated_mix__sliding_block_cached__moe_arch_mod__decode'

def setup_inputs():
    _rng = _Rng(jax.random.key(int.from_bytes(__import__("os").urandom(4), "little")))
    _w = (lambda a: (lambda t: t.astype(jnp.bfloat16) if jnp.issubdtype(t.dtype, jnp.floating) else t)(jnp.asarray(a)))
    def _A_setup():
        B, Sq, D = 1, 1, 640
        Hq, Hkv, Sk, Dh = 32, 32, 32768, 192
        assert Hq % Hkv == 0, (Hq, Hkv)
        return {
            "x": _w((lambda *s: _rng.normal(s) * 0.05)(B, Sq, D)),
            "k_cache": _w((lambda *s: _rng.normal(s) * 0.05)(B, Hkv, Sk, Dh)),
            "v_cache": _w((lambda *s: _rng.normal(s) * 0.05)(B, Hkv, Sk, Dh)),
            "wq": _w((lambda *s: _rng.normal(s) * 0.05)(D, Hq * Dh) * (D ** -0.5)),
            "wo": _w((lambda *s: _rng.normal(s) * 0.05)(Hq * Dh, D) * ((Hq * Dh) ** -0.5)),
        }
    _A_in = _A_setup()

    def _B_setup():
        B, S, D, F, C = 1, 1, 640, 1536, 1
        return {
            "x": _w((lambda *s: _rng.normal(s) * 0.05)(B, S, D)),
            "w_r": _w((lambda *s: _rng.normal(s) * 0.05)(D)),
            "w_gate": _w((lambda *s: _rng.normal(s) * 0.05)(D, F)),
            "w_up": _w((lambda *s: _rng.normal(s) * 0.05)(D, F)),
            "w_down": _w((lambda *s: _rng.normal(s) * 0.05)(F, D)),
        }
    _B_in = _B_setup()

    return {
        "A_x": _A_in["x"],
        "A_k_cache": _A_in["k_cache"],
        "A_v_cache": _A_in["v_cache"],
        "A_wq": _A_in["wq"],
        "A_wo": _A_in["wo"],
        "B_x": _B_in["x"],
        "B_w_r": _B_in["w_r"],
        "B_w_gate": _B_in["w_gate"],
        "B_w_up": _B_in["w_up"],
        "B_w_down": _B_in["w_down"],
        "gate_w": _w((lambda *s: _rng.normal(s) * 0.05)(640)),
    }

def reference(A_x, A_k_cache, A_v_cache, A_wq, A_wo, B_x, B_w_r, B_w_gate, B_w_up, B_w_down, gate_w):
    def _A_ref(x, k_cache, v_cache, wq, wo):
        B, Sq, D = x.shape
        Hq, Dh = 32, 192
        Hkv, Sk = k_cache.shape[1], k_cache.shape[2]
        W = min(4096, max(256, Sk // 4))
        rep = Hq // Hkv
        q = (lambda x, *d: x.transpose(*d))((x @ wq).reshape(B, Sq, Hq, Dh), 0, 2, 1, 3)
        k = jnp.repeat(k_cache[:, :, Sk - W:, :], rep, axis=1)
        v = jnp.repeat(v_cache[:, :, Sk - W:, :], rep, axis=1)
        scores = jnp.einsum("bhqd,bhkd->bhqk", q, k) * (Dh ** -0.5)
        p = _softmax(scores, axis=-1)
        o = jnp.einsum("bhqk,bhkd->bhqd", p, v)
        return (lambda x, *d: x.transpose(*d))(o, 0, 2, 1, 3).reshape(B, Sq, Hq * Dh) @ wo

    def _B_ref(x, w_r, w_gate, w_up, w_down):
        B, S, D = x.shape
        C = 1
        r = x @ w_r
        idx = jnp.argsort(-r, axis=-1)[:, :C]
        idx_e = jnp.repeat(idx.reshape(B, C, 1), D, axis=2)
        x_sel = jnp.take_along_axis(x, idx_e, axis=1)
        g = _silu(x_sel @ w_gate)
        u = x_sel @ w_up
        y = (g * u) @ w_down
        r_sel = _sigmoid(jnp.take_along_axis(r, idx, axis=1))
        y = y * r_sel.reshape(B, C, 1)
        b_off = (jnp.arange(B) * S).reshape(B, 1)
        flat_idx = (idx + b_off).reshape(B * C)
        zero = (x * 0.0).reshape(B * S, D)
        upd = _scatter_add(zero, flat_idx, y.reshape(B * C, D), axis=0)
        return x + upd.reshape(B, S, D)

    x = A_x
    g = _sigmoid((x * gate_w).sum(-1, keepdims=True))
    a = _A_ref(x, A_k_cache, A_v_cache, A_wq, A_wo)
    b = _B_ref(x, B_w_r, B_w_gate, B_w_up, B_w_down)
    return g * a + (1 - g) * b
```

```python
import functools

import jax
import jax.numpy as jnp
import jax.experimental.pallas as pl
import jax.experimental.pallas.tpu as pltpu

_HQ, _DH = 32, 192
_PAIR = 2 * _DH
_NPAIR = _HQ // 2
_DEPTH = 4
_ROWS = 16
_WO_CHUNKS = 16


def _kernel(x_hbm, k_hbm, v_hbm, wq_hbm, wo_hbm, wr_hbm, wg_hbm, wu_hbm, wd_hbm, gw_hbm,
            out_hbm,
            x_v, wr_v, gw_v, wq_v, wo_v, wg_v, wu_v, wd_v, k_buf, v_buf, qd_ref, o_ref, out_v,
            small_sems, w_sems, wo_sems, k_sems, v_sems, *, sk, w):
    f32, bf16 = jnp.float32, jnp.bfloat16
    col0 = sk - w
    wo_rows = wo_v.shape[0] // _WO_CHUNKS

    def k_copy(j, slot):
        r = pl.multiple_of(j * _PAIR, _PAIR)
        return pltpu.make_async_copy(
            k_hbm.at[pl.ds(r, _PAIR), pl.ds(col0, w)], k_buf.at[slot], k_sems.at[slot])

    def v_copy(j, slot):
        r = pl.multiple_of(j * _PAIR, _PAIR)
        return pltpu.make_async_copy(
            v_hbm.at[pl.ds(r, _PAIR), pl.ds(col0, w)], v_buf.at[slot], v_sems.at[slot])

    def wo_copy(c):
        return pltpu.make_async_copy(
            wo_hbm.at[pl.ds(c * wo_rows, wo_rows)], wo_v.at[pl.ds(c * wo_rows, wo_rows)],
            wo_sems.at[c])

    x_cp = pltpu.make_async_copy(x_hbm.at[0], x_v, small_sems.at[0])
    wr_cp = pltpu.make_async_copy(wr_hbm, wr_v, small_sems.at[1])
    gw_cp = pltpu.make_async_copy(gw_hbm, gw_v, small_sems.at[2])
    wq_cp = pltpu.make_async_copy(wq_hbm, wq_v, w_sems.at[0])
    wg_cp = pltpu.make_async_copy(wg_hbm, wg_v, w_sems.at[1])
    wu_cp = pltpu.make_async_copy(wu_hbm, wu_v, w_sems.at[2])
    wd_cp = pltpu.make_async_copy(wd_hbm, wd_v, w_sems.at[3])
    out_cp = pltpu.make_async_copy(out_v, out_hbm.at[0], small_sems.at[3])

    wq_cp.start()
    x_cp.start()
    wr_cp.start()
    gw_cp.start()
    for j in range(_DEPTH):
        k_copy(j, j).start()
        v_copy(j, j).start()

    rows = jax.lax.broadcasted_iota(jnp.int32, (_ROWS, _PAIR), 0)
    cols = jax.lax.broadcasted_iota(jnp.int32, (_ROWS, _PAIR), 1)
    own = (cols >= _DH) == ((rows & 1) == 1)

    x_cp.wait()
    x = x_v[...]
    xb = jnp.broadcast_to(x, (_ROWS, x.shape[1]))

    wq_cp.wait()
    for j in range(_NPAIR):
        q = jnp.dot(xb, wq_v[:, j * _PAIR:(j + 1) * _PAIR], preferred_element_type=f32)
        qd_ref[j] = jnp.where(own, q, 0.0).astype(bf16)

    scale = _DH ** -0.5

    def pair(j, carry):
        slot = j % _DEPTH
        k_copy(j, slot).wait()
        s = jnp.dot(qd_ref[j], k_buf[slot], preferred_element_type=f32) * scale
        m = jnp.max(s, axis=1, keepdims=True)
        p = jnp.exp(s - m)
        l = jnp.sum(p, axis=1, keepdims=True)
        v_copy(j, slot).wait()
        o = jax.lax.dot_general(p.astype(bf16), v_buf[slot], (((1,), (1,)), ((), ())),
                                preferred_element_type=f32)
        nxt = j + _DEPTH

        @pl.when(nxt < _NPAIR)
        def _():
            k_copy(nxt, slot).start()
            v_copy(nxt, slot).start()

        @pl.when(nxt == _NPAIR)
        def _():
            wg_cp.start()
            wu_cp.start()
            wd_cp.start()
            for c in range(_WO_CHUNKS):
                wo_copy(c).start()

        o = jnp.where(own, o / l, 0.0)
        o_ref[j] = (o[0:1] + o[1:2]).astype(bf16)
        return carry

    jax.lax.fori_loop(0, _NPAIR, pair, 0)

    wr_cp.wait()
    gw_cp.wait()
    xf = x.astype(f32)
    r = jnp.sum(xf * wr_v[...].astype(f32).reshape(1, -1), axis=1, keepdims=True)
    gate = jax.nn.sigmoid(jnp.sum(xf * gw_v[...].astype(f32).reshape(1, -1), axis=1, keepdims=True))
    wg_cp.wait()
    hg = jnp.dot(xb, wg_v[...], preferred_element_type=f32)
    wu_cp.wait()
    hu = jnp.dot(xb, wu_v[...], preferred_element_type=f32)
    h = (jax.nn.silu(hg) * hu).astype(bf16)
    wd_cp.wait()
    y = jnp.dot(h, wd_v[...], preferred_element_type=f32)[0:1]
    b = xf + (xf * 0.0 + y * jax.nn.sigmoid(r))

    per = wo_rows // _PAIR
    acc = jnp.zeros((_ROWS, x.shape[1]), f32)
    for c in range(_WO_CHUNKS):
        wo_copy(c).wait()
        for i in range(per):
            j = c * per + i
            ob = jnp.broadcast_to(o_ref[j], (_ROWS, _PAIR))
            acc += jnp.dot(ob, wo_v[j * _PAIR:(j + 1) * _PAIR, :], preferred_element_type=f32)
    a = acc[0:1]

    out_v[...] = (gate * a + (1.0 - gate) * b).astype(out_v.dtype)
    out_cp.start()
    out_cp.wait()


@jax.jit
def pallas_gated_mix__sliding_block_cached__moe_arch_mod__decode_kernel(
    A_x: jax.Array,
    A_k_cache: jax.Array,
    A_v_cache: jax.Array,
    A_wq: jax.Array,
    A_wo: jax.Array,
    B_x: jax.Array,
    B_w_r: jax.Array,
    B_w_gate: jax.Array,
    B_w_up: jax.Array,
    B_w_down: jax.Array,
    gate_w: jax.Array,
):
    del B_x
    b, sq, d = A_x.shape
    _, hkv, sk, dh = A_k_cache.shape
    assert (b, sq, hkv, dh) == (1, 1, _HQ, _DH)
    w = min(4096, max(256, sk // 4))
    dt = A_x.dtype
    kt = jnp.swapaxes(A_k_cache, 2, 3).reshape(hkv * dh, sk)
    vt = jnp.swapaxes(A_v_cache, 2, 3).reshape(hkv * dh, sk)

    hbm = pl.BlockSpec(memory_space=pl.ANY)
    vmem = pltpu.VMEM
    dma = pltpu.SemaphoreType.DMA
    return pl.pallas_call(
        functools.partial(_kernel, sk=sk, w=w),
        in_specs=[hbm] * 10,
        out_specs=hbm,
        out_shape=jax.ShapeDtypeStruct((b, sq, d), dt),
        scratch_shapes=[
            vmem((1, d), dt), vmem(B_w_r.shape, dt), vmem(gate_w.shape, dt),
            vmem(A_wq.shape, dt), vmem(A_wo.shape, dt),
            vmem(B_w_gate.shape, dt), vmem(B_w_up.shape, dt), vmem(B_w_down.shape, dt),
            vmem((_DEPTH, _PAIR, w), dt), vmem((_DEPTH, _PAIR, w), dt),
            vmem((_NPAIR, _ROWS, _PAIR), dt), vmem((_NPAIR, 1, _PAIR), dt),
            vmem((1, d), dt),
            dma((4,)), dma((4,)), dma((_WO_CHUNKS,)), dma((_DEPTH,)), dma((_DEPTH,)),
        ],
        compiler_params=pltpu.CompilerParams(vmem_limit_bytes=100 * 1024 * 1024),
    )(A_x, kt, vt, A_wq, A_wo, B_w_r, B_w_gate, B_w_up, B_w_down, gate_w)
```

```python
import functools

import jax
import jax.numpy as jnp
import jax.experimental.pallas as pl
import jax.experimental.pallas.tpu as pltpu

_HQ, _DH = 32, 192
_PAIR = 2 * _DH
_NPAIR = _HQ // 2
_ROWS = 16
_T = 16
_KVC = 1024
_WQC = 1024
_WR = 32
_WO_GROUPS = (3072, 1536, 768, 384, 256, 128)
_WO_EARLY = 1


def _kernel(x_hbm, k_hbm, v_hbm, wq_hbm, wo_hbm, wr_hbm, wg_hbm, wu_hbm, wd_hbm, gw_hbm,
            out_hbm,
            x_v, wr_v, gw_v, wq_v, wo_v, wg_v, wu_v, wd_v, k_buf, v_buf, qd_ref, o_ref, out_v,
            small_sems, w_sems, wo_sems, kv_sems, *, sk, w):
    f32, bf16 = jnp.float32, jnp.bfloat16
    col0 = sk - w
    d = x_v.shape[1]
    copy = pltpu.make_async_copy

    def whole(buf, sem):
        return copy(buf, buf, sem)

    def start_kv(j, slot, lo, hi):
        def body(t, c):
            r = pl.multiple_of(t * _T, _T)
            src_r = pl.multiple_of(j * _PAIR + r, _T)
            for cc in range(w // _KVC):
                src = (pl.ds(src_r, _T), pl.ds(col0 + cc * _KVC, _KVC))
                dst = (slot, pl.ds(r, _T), pl.ds(cc * _KVC, _KVC))
                copy(k_hbm.at[src], k_buf.at[dst], kv_sems.at[0, slot]).start(priority=0)
                copy(v_hbm.at[src], v_buf.at[dst], kv_sems.at[1, slot]).start(priority=1)
            return c
        jax.lax.fori_loop(lo, hi, body, 0)

    def start_rows(src, dst, sem, lo, hi):
        half = (hi - lo) // 2
        def body(t, c):
            r0 = pl.multiple_of(lo + t * _WR, _WR)
            r1 = pl.multiple_of(lo + half + t * _WR, _WR)
            copy(src.at[pl.ds(r0, _WR)], dst.at[pl.ds(r0, _WR)], sem).start(priority=0)
            copy(src.at[pl.ds(r1, _WR)], dst.at[pl.ds(r1, _WR)], sem).start(priority=1)
            return c
        jax.lax.fori_loop(0, half // _WR, body, 0)

    wo_lo = [sum(_WO_GROUPS[:g]) for g in range(len(_WO_GROUPS) + 1)]

    def start_wo(g):
        start_rows(wo_hbm, wo_v, wo_sems.at[g], wo_lo[g], wo_lo[g + 1])

    x_cp = copy(x_hbm.at[0], x_v, small_sems.at[0])
    wr_cp = copy(wr_hbm, wr_v, small_sems.at[1])
    gw_cp = copy(gw_hbm, gw_v, small_sems.at[2])
    out_cp = copy(out_v, out_hbm.at[0], small_sems.at[3])

    x_cp.start()
    wr_cp.start()
    gw_cp.start()

    def gu_body(t, c):
        r = pl.ds(pl.multiple_of(t * _T, _T), _T)
        copy(wg_hbm.at[r], wg_v.at[r], w_sems.at[0]).start(priority=0)
        copy(wu_hbm.at[r], wu_v.at[r], w_sems.at[0]).start(priority=1)
        return c
    jax.lax.fori_loop(0, wg_v.shape[0] // _T, gu_body, 0)
    start_rows(wd_hbm, wd_v, w_sems.at[1], 0, wd_v.shape[0])

    def wq_body(t, c):
        half = wq_v.shape[0] // 2
        r0 = pl.ds(pl.multiple_of(t * _T, _T), _T)
        r1 = pl.ds(pl.multiple_of(half + t * _T, _T), _T)
        for cc in range(wq_v.shape[1] // _WQC):
            cs = pl.ds(cc * _WQC, _WQC)
            copy(wq_hbm.at[r0, cs], wq_v.at[r0, cs], w_sems.at[2]).start(priority=0)
            copy(wq_hbm.at[r1, cs], wq_v.at[r1, cs], w_sems.at[2]).start(priority=1)
        return c
    jax.lax.fori_loop(0, wq_v.shape[0] // (2 * _T), wq_body, 0)

    x_cp.wait()
    wr_cp.wait()
    gw_cp.wait()
    x = x_v[...]
    xb = jnp.broadcast_to(x, (_ROWS, d))
    xf = x.astype(f32)
    r = jnp.sum(xf * wr_v[...].astype(f32).reshape(1, -1), axis=1, keepdims=True)
    gate = jax.nn.sigmoid(jnp.sum(xf * gw_v[...].astype(f32).reshape(1, -1), axis=1, keepdims=True))
    whole(wg_v, w_sems.at[0]).wait()
    whole(wu_v, w_sems.at[0]).wait()
    hg = jnp.dot(xb, wg_v[...], preferred_element_type=f32)
    hu = jnp.dot(xb, wu_v[...], preferred_element_type=f32)
    h = (jax.nn.silu(hg) * hu).astype(bf16)
    whole(wd_v, w_sems.at[1]).wait()
    y = jnp.dot(h, wd_v[...], preferred_element_type=f32)[0:1]
    b_part = (1.0 - gate) * (xf + (xf * 0.0 + y * jax.nn.sigmoid(r)))

    ntile = _PAIR // _T
    start_kv(0, 0, 0, ntile)

    rows = jax.lax.broadcasted_iota(jnp.int32, (_ROWS, _PAIR), 0)
    cols = jax.lax.broadcasted_iota(jnp.int32, (_ROWS, _PAIR), 1)
    own = (cols >= _DH) == ((rows & 1) == 1)

    whole(wq_v, w_sems.at[2]).wait()
    for j in range(_NPAIR):
        q = jnp.dot(xb, wq_v[:, j * _PAIR:(j + 1) * _PAIR], preferred_element_type=f32)
        qd_ref[j] = jnp.where(own, q, 0.0).astype(bf16)

    scale = _DH ** -0.5

    def pair(j, carry):
        slot = j % 2

        @pl.when(j + 1 < _NPAIR)
        def _():
            start_kv(j + 1, 1 - slot, 0, ntile)

        @pl.when(j + 1 == _NPAIR)
        def _():
            for g in range(_WO_EARLY):
                start_wo(g)

        whole(k_buf.at[slot], kv_sems.at[0, slot]).wait()
        s = jnp.dot(qd_ref[j], k_buf[slot], preferred_element_type=f32) * scale
        m = jnp.max(s, axis=1, keepdims=True)
        p = jnp.exp(s - m)
        l = jnp.sum(p, axis=1, keepdims=True)
        whole(v_buf.at[slot], kv_sems.at[1, slot]).wait()
        o = jax.lax.dot_general(p.astype(bf16), v_buf[slot], (((1,), (1,)), ((), ())),
                                preferred_element_type=f32)
        o = jnp.where(own, o / l, 0.0)
        o_ref[j] = (o[0:1] + o[1:2]).astype(bf16)
        return carry

    jax.lax.fori_loop(0, _NPAIR, pair, 0)

    for g in range(_WO_EARLY, len(_WO_GROUPS)):
        start_wo(g)

    acc = jnp.zeros((_ROWS, d), f32)
    for g, n in enumerate(_WO_GROUPS):
        lo = wo_lo[g]
        whole(wo_v.at[pl.ds(lo, n)], wo_sems.at[g]).wait()
        for r0 in range(lo, lo + n, 128):
            j, c = divmod(r0, _PAIR)
            ob = jnp.broadcast_to(o_ref[j, :, c:c + 128], (_ROWS, 128))
            acc += jnp.dot(ob, wo_v[r0:r0 + 128, :], preferred_element_type=f32)

    out_v[...] = (gate * acc[0:1] + b_part).astype(out_v.dtype)
    out_cp.start()
    out_cp.wait()


@jax.jit
def pallas_gated_mix__sliding_block_cached__moe_arch_mod__decode_kernel(
    A_x: jax.Array,
    A_k_cache: jax.Array,
    A_v_cache: jax.Array,
    A_wq: jax.Array,
    A_wo: jax.Array,
    B_x: jax.Array,
    B_w_r: jax.Array,
    B_w_gate: jax.Array,
    B_w_up: jax.Array,
    B_w_down: jax.Array,
    gate_w: jax.Array,
):
    del B_x
    b, sq, d = A_x.shape
    _, hkv, sk, dh = A_k_cache.shape
    assert (b, sq, hkv, dh) == (1, 1, _HQ, _DH)
    w = min(4096, max(256, sk // 4))
    dt = A_x.dtype
    kt = jnp.swapaxes(A_k_cache, 2, 3).reshape(hkv * dh, sk)
    vt = jnp.swapaxes(A_v_cache, 2, 3).reshape(hkv * dh, sk)

    hbm = pl.BlockSpec(memory_space=pl.ANY)
    vmem = pltpu.VMEM
    dma = pltpu.SemaphoreType.DMA
    return pl.pallas_call(
        functools.partial(_kernel, sk=sk, w=w),
        in_specs=[hbm] * 10,
        out_specs=hbm,
        out_shape=jax.ShapeDtypeStruct((b, sq, d), dt),
        scratch_shapes=[
            vmem((1, d), dt), vmem(B_w_r.shape, dt), vmem(gate_w.shape, dt),
            vmem(A_wq.shape, dt), vmem(A_wo.shape, dt),
            vmem(B_w_gate.shape, dt), vmem(B_w_up.shape, dt), vmem(B_w_down.shape, dt),
            vmem((2, _PAIR, w), dt), vmem((2, _PAIR, w), dt),
            vmem((_NPAIR, _ROWS, _PAIR), dt), vmem((_NPAIR, 1, _PAIR), dt),
            vmem((1, d), dt),
            dma((4,)), dma((3,)), dma((len(_WO_GROUPS),)), dma((2, 2)),
        ],
        compiler_params=pltpu.CompilerParams(vmem_limit_bytes=100 * 1024 * 1024),
    )(A_x, kt, vt, A_wq, A_wo, B_w_r, B_w_gate, B_w_up, B_w_down, gate_w)
```

```python
import functools

import jax
import jax.numpy as jnp
import jax.experimental.pallas as pl
import jax.experimental.pallas.tpu as pltpu

_HQ, _DH = 32, 192
_PAIR = 2 * _DH
_NPAIR = _HQ // 2
_ROWS = 16
_T = 16
_KVR, _KVC, _KVB = 32, 512, 3
_WQC = 2048
_WR = 32
_WO_GROUPS = (3072, 1536, 768, 384, 256, 128)
_WO_EARLY = 1


def _kernel(x_hbm, k_hbm, v_hbm, wq_hbm, wo_hbm, wr_hbm, wg_hbm, wu_hbm, wd_hbm, gw_hbm,
            out_hbm,
            x_v, wr_v, gw_v, wq_v, wo_v, wg_v, wu_v, wd_v, k_buf, v_buf, qd_ref, o_ref, out_v,
            small_sems, w_sems, wo_sems, kv_sems, *, sk, w):
    f32, bf16 = jnp.float32, jnp.bfloat16
    col0 = sk - w
    d = x_v.shape[1]
    copy = pltpu.make_async_copy

    def whole(buf, sem):
        return copy(buf, buf, sem)

    def start_kv(j, slot):
        def body(blk, c):
            for cc in range(w // _KVC):
                for t in range(_KVB):
                    r = pl.multiple_of((blk * _KVB + t) * _KVR, _KVR)
                    src = (pl.ds(pl.multiple_of(j * _PAIR + r, _KVR), _KVR),
                           pl.ds(col0 + cc * _KVC, _KVC))
                    dst = (slot, pl.ds(r, _KVR), pl.ds(cc * _KVC, _KVC))
                    copy(k_hbm.at[src], k_buf.at[dst], kv_sems.at[0, slot]).start(priority=0)
                    copy(v_hbm.at[src], v_buf.at[dst], kv_sems.at[1, slot]).start(priority=1)
            return c
        jax.lax.fori_loop(0, _PAIR // (_KVB * _KVR), body, 0)

    def start_rows(src, dst, sem, lo, hi):
        half = (hi - lo) // 2
        def body(t, c):
            r0 = pl.multiple_of(lo + t * _WR, _WR)
            r1 = pl.multiple_of(lo + half + t * _WR, _WR)
            copy(src.at[pl.ds(r0, _WR)], dst.at[pl.ds(r0, _WR)], sem).start(priority=0)
            copy(src.at[pl.ds(r1, _WR)], dst.at[pl.ds(r1, _WR)], sem).start(priority=1)
            return c
        jax.lax.fori_loop(0, half // _WR, body, 0)

    wo_lo = [sum(_WO_GROUPS[:g]) for g in range(len(_WO_GROUPS) + 1)]

    def start_wo(g):
        start_rows(wo_hbm, wo_v, wo_sems.at[g], wo_lo[g], wo_lo[g + 1])

    x_cp = copy(x_hbm.at[0], x_v, small_sems.at[0])
    wr_cp = copy(wr_hbm, wr_v, small_sems.at[1])
    gw_cp = copy(gw_hbm, gw_v, small_sems.at[2])
    out_cp = copy(out_v, out_hbm.at[0], small_sems.at[3])

    x_cp.start()
    wr_cp.start()
    gw_cp.start()

    def gu_body(t, c):
        r = pl.ds(pl.multiple_of(t * _T, _T), _T)
        copy(wg_hbm.at[r], wg_v.at[r], w_sems.at[0]).start(priority=0)
        copy(wu_hbm.at[r], wu_v.at[r], w_sems.at[0]).start(priority=1)
        return c
    jax.lax.fori_loop(0, wg_v.shape[0] // _T, gu_body, 0)
    start_rows(wd_hbm, wd_v, w_sems.at[1], 0, wd_v.shape[0])

    def wq_body(t, c):
        half = wq_v.shape[0] // 2
        r0 = pl.ds(pl.multiple_of(t * 8, 8), 8)
        r1 = pl.ds(pl.multiple_of(half + t * 8, 8), 8)
        for cc in range(wq_v.shape[1] // _WQC):
            cs = pl.ds(cc * _WQC, _WQC)
            copy(wq_hbm.at[r0, cs], wq_v.at[r0, cs], w_sems.at[2]).start(priority=0)
            copy(wq_hbm.at[r1, cs], wq_v.at[r1, cs], w_sems.at[2]).start(priority=1)
        return c
    jax.lax.fori_loop(0, wq_v.shape[0] // 16, wq_body, 0)

    x_cp.wait()
    wr_cp.wait()
    gw_cp.wait()
    x = x_v[...]
    xb = jnp.broadcast_to(x, (_ROWS, d))
    xf = x.astype(f32)
    r = jnp.sum(xf * wr_v[...].astype(f32).reshape(1, -1), axis=1, keepdims=True)
    gate = jax.nn.sigmoid(jnp.sum(xf * gw_v[...].astype(f32).reshape(1, -1), axis=1, keepdims=True))
    whole(wg_v, w_sems.at[0]).wait()
    whole(wu_v, w_sems.at[0]).wait()
    hg = jnp.dot(xb, wg_v[...], preferred_element_type=f32)
    hu = jnp.dot(xb, wu_v[...], preferred_element_type=f32)
    h = (jax.nn.silu(hg) * hu).astype(bf16)
    whole(wd_v, w_sems.at[1]).wait()
    y = jnp.dot(h, wd_v[...], preferred_element_type=f32)[0:1]
    b_part = (1.0 - gate) * (xf + (xf * 0.0 + y * jax.nn.sigmoid(r)))

    start_kv(0, 0)

    rows = jax.lax.broadcasted_iota(jnp.int32, (_ROWS, _PAIR), 0)
    cols = jax.lax.broadcasted_iota(jnp.int32, (_ROWS, _PAIR), 1)
    own = (cols >= _DH) == ((rows & 1) == 1)

    whole(wq_v, w_sems.at[2]).wait()
    for j in range(_NPAIR):
        q = jnp.dot(xb, wq_v[:, j * _PAIR:(j + 1) * _PAIR], preferred_element_type=f32)
        qd_ref[j] = jnp.where(own, q, 0.0).astype(bf16)

    scale = _DH ** -0.5

    def pair(j, carry):
        slot = j % 2

        @pl.when(j + 1 < _NPAIR)
        def _():
            start_kv(j + 1, 1 - slot)

        @pl.when(j + 1 == _NPAIR)
        def _():
            for g in range(_WO_EARLY):
                start_wo(g)

        whole(k_buf.at[slot], kv_sems.at[0, slot]).wait()
        s = jnp.dot(qd_ref[j], k_buf[slot], preferred_element_type=f32) * scale
        m = jnp.max(s, axis=1, keepdims=True)
        p = jnp.exp(s - m)
        l = jnp.sum(p, axis=1, keepdims=True)
        whole(v_buf.at[slot], kv_sems.at[1, slot]).wait()
        o = jax.lax.dot_general(p.astype(bf16), v_buf[slot], (((1,), (1,)), ((), ())),
                                preferred_element_type=f32)
        o = jnp.where(own, o / l, 0.0)
        o_ref[j] = (o[0:1] + o[1:2]).astype(bf16)
        return carry

    jax.lax.fori_loop(0, _NPAIR, pair, 0)

    for g in range(_WO_EARLY, len(_WO_GROUPS)):
        start_wo(g)

    acc = jnp.zeros((_ROWS, d), f32)
    for g, n in enumerate(_WO_GROUPS):
        lo = wo_lo[g]
        whole(wo_v.at[pl.ds(lo, n)], wo_sems.at[g]).wait()
        for r0 in range(lo, lo + n, 128):
            j, c = divmod(r0, _PAIR)
            ob = jnp.broadcast_to(o_ref[j, :, c:c + 128], (_ROWS, 128))
            acc += jnp.dot(ob, wo_v[r0:r0 + 128, :], preferred_element_type=f32)

    out_v[...] = (gate * acc[0:1] + b_part).astype(out_v.dtype)
    out_cp.start()
    out_cp.wait()


@jax.jit
def pallas_gated_mix__sliding_block_cached__moe_arch_mod__decode_kernel(
    A_x: jax.Array,
    A_k_cache: jax.Array,
    A_v_cache: jax.Array,
    A_wq: jax.Array,
    A_wo: jax.Array,
    B_x: jax.Array,
    B_w_r: jax.Array,
    B_w_gate: jax.Array,
    B_w_up: jax.Array,
    B_w_down: jax.Array,
    gate_w: jax.Array,
):
    del B_x
    b, sq, d = A_x.shape
    _, hkv, sk, dh = A_k_cache.shape
    assert (b, sq, hkv, dh) == (1, 1, _HQ, _DH)
    w = min(4096, max(256, sk // 4))
    dt = A_x.dtype
    kt = jnp.swapaxes(A_k_cache, 2, 3).reshape(hkv * dh, sk)
    vt = jnp.swapaxes(A_v_cache, 2, 3).reshape(hkv * dh, sk)

    hbm = pl.BlockSpec(memory_space=pl.ANY)
    vmem = pltpu.VMEM
    dma = pltpu.SemaphoreType.DMA
    return pl.pallas_call(
        functools.partial(_kernel, sk=sk, w=w),
        in_specs=[hbm] * 10,
        out_specs=hbm,
        out_shape=jax.ShapeDtypeStruct((b, sq, d), dt),
        scratch_shapes=[
            vmem((1, d), dt), vmem(B_w_r.shape, dt), vmem(gate_w.shape, dt),
            vmem(A_wq.shape, dt), vmem(A_wo.shape, dt),
            vmem(B_w_gate.shape, dt), vmem(B_w_up.shape, dt), vmem(B_w_down.shape, dt),
            vmem((2, _PAIR, w), dt), vmem((2, _PAIR, w), dt),
            vmem((_NPAIR, _ROWS, _PAIR), dt), vmem((_NPAIR, 1, _PAIR), dt),
            vmem((1, d), dt),
            dma((4,)), dma((3,)), dma((len(_WO_GROUPS),)), dma((2, 2)),
        ],
        compiler_params=pltpu.CompilerParams(
            vmem_limit_bytes=100 * 1024 * 1024,
            disable_bounds_checks=True, disable_semaphore_checks=True),
    )(A_x, kt, vt, A_wq, A_wo, B_w_r, B_w_gate, B_w_up, B_w_down, gate_w)
```

```python
import functools

import jax
import jax.numpy as jnp
import jax.experimental.pallas as pl
import jax.experimental.pallas.tpu as pltpu

_HQ, _DH = 32, 192
_PAIR = 2 * _DH
_NPAIR = _HQ // 2
_ROWS = 16
_T = 8

_KV_R, _KV_C, _KV_B = 32, 512, 3
_Q_C, _Q_G = 2048, 4
_GU_G = 4
_W_R, _D_G = 32, 2
_WO_GROUPS = (
    (512, (0, 1024, 2048), (3072, 4096, 5120)),
    (256, (512, 1536, 2560), (3584, 4608, 5632)),
    (128, (768, 1792, 2816), (3840, 4864, 5888)),
    (64, (896, 1920, 2944), (960, 1984, 3008)),
    (64, (3968, 4992), (4032, 5056)),
    (64, (6016,), (6080,)),
)


def _wo_chunks(group):
    n, p0, p1 = group
    rows = sorted(a + i for a in (*p0, *p1) for i in range(n))
    chunks = rows[::128]
    assert all(c % 128 == 0 for c in chunks)
    assert [c + i for c in chunks for i in range(128)] == rows
    return chunks


def _kernel(x_hbm, k_hbm, v_hbm, wq_hbm, wo_hbm, wr_hbm, wg_hbm, wu_hbm, wd_hbm, gw_hbm,
            out_hbm,
            x_v, wr_v, gw_v, wq_v, wo_v, wg_v, wu_v, wd_v, k_buf, v_buf, qd_ref, o_ref, out_v,
            small_sems, w_sems, wo_sems, kv_sems, *, col0):
    f32, bf16 = jnp.float32, jnp.bfloat16
    d = x_v.shape[1]
    w = k_buf.shape[2]
    copy = pltpu.make_async_copy

    def wait_all(buf, sem):
        copy(buf, buf, sem).wait()

    def rows(start, n):
        return pl.ds(pl.multiple_of(start, n), n)

    def start_row_pieces(src, dst, sem, n, starts0, starts1):
        def body(t, c):
            for a, b in zip(starts0, starts1, strict=True):
                r0, r1 = rows(a + t * _W_R, _W_R), rows(b + t * _W_R, _W_R)
                copy(src.at[r0], dst.at[r0], sem).start(priority=0)
                copy(src.at[r1], dst.at[r1], sem).start(priority=1)
            return c
        jax.lax.fori_loop(0, n // _W_R, body, 0)

    def start_kv(j, slot):
        def body(blk, c):
            for cc in range(w // _KV_C):
                for t in range(_KV_B):
                    r = (blk * _KV_B + t) * _KV_R
                    src = (rows(j * _PAIR + r, _KV_R), pl.ds(col0 + cc * _KV_C, _KV_C))
                    dst = (slot, rows(r, _KV_R), pl.ds(cc * _KV_C, _KV_C))
                    copy(k_hbm.at[src], k_buf.at[dst], kv_sems.at[0, slot]).start(priority=0)
                    copy(v_hbm.at[src], v_buf.at[dst], kv_sems.at[1, slot]).start(priority=1)
            return c
        jax.lax.fori_loop(0, _PAIR // (_KV_B * _KV_R), body, 0)

    def start_wo(g):
        start_row_pieces(wo_hbm, wo_v, wo_sems.at[g], *_WO_GROUPS[g])

    x_cp = copy(x_hbm.at[0], x_v, small_sems.at[0])
    wr_cp = copy(wr_hbm, wr_v, small_sems.at[1])
    gw_cp = copy(gw_hbm, gw_v, small_sems.at[2])
    out_cp = copy(out_v, out_hbm.at[0], small_sems.at[3])
    wg_sem, wu_sem, wd_sem, wq_sem = (w_sems.at[i] for i in range(4))

    x_cp.start()
    wr_cp.start()
    gw_cp.start()

    def gu_body(t, c):
        reg = wg_v.shape[0] // _GU_G
        for g in range(_GU_G):
            r = rows(g * reg + t * _T, _T)
            copy(wg_hbm.at[r], wg_v.at[r], wg_sem).start(priority=0)
            copy(wu_hbm.at[r], wu_v.at[r], wu_sem).start(priority=1)
        return c
    jax.lax.fori_loop(0, wg_v.shape[0] // (_T * _GU_G), gu_body, 0)

    reg = wd_v.shape[0] // (2 * _D_G)
    start_row_pieces(wd_hbm, wd_v, wd_sem, reg, [g * reg for g in range(_D_G)],
                     [(_D_G + g) * reg for g in range(_D_G)])

    def wq_body(t, c):
        reg = wq_v.shape[0] // (2 * _Q_G)
        for cc in range(wq_v.shape[1] // _Q_C):
            cs = pl.ds(cc * _Q_C, _Q_C)
            for g in range(_Q_G):
                r0, r1 = rows(g * reg + t * _T, _T), rows((_Q_G + g) * reg + t * _T, _T)
                copy(wq_hbm.at[r0, cs], wq_v.at[r0, cs], wq_sem).start(priority=0)
                copy(wq_hbm.at[r1, cs], wq_v.at[r1, cs], wq_sem).start(priority=1)
        return c
    jax.lax.fori_loop(0, wq_v.shape[0] // (2 * _Q_G * _T), wq_body, 0)

    x_cp.wait()
    wr_cp.wait()
    gw_cp.wait()
    x = x_v[...]
    xb = jnp.broadcast_to(x, (_ROWS, d))
    xf = x.astype(f32)
    r = jnp.sum(xf * wr_v[...].astype(f32).reshape(1, d), axis=1, keepdims=True)
    gate = jax.nn.sigmoid(jnp.sum(xf * gw_v[...].astype(f32).reshape(1, d), axis=1, keepdims=True))
    wait_all(wg_v, wg_sem)
    hg = jnp.dot(xb, wg_v[...], preferred_element_type=f32)
    wait_all(wu_v, wu_sem)
    hu = jnp.dot(xb, wu_v[...], preferred_element_type=f32)
    h = (jax.nn.silu(hg) * hu).astype(bf16)
    wait_all(wd_v, wd_sem)
    y = jnp.dot(h, wd_v[...], preferred_element_type=f32)[0:1]
    b_part = (1.0 - gate) * (xf + (xf * 0.0 + y * jax.nn.sigmoid(r)))

    start_kv(0, 0)

    row_id = jax.lax.broadcasted_iota(jnp.int32, (_ROWS, _PAIR), 0)
    col_id = jax.lax.broadcasted_iota(jnp.int32, (_ROWS, _PAIR), 1)
    own = (col_id >= _DH) == ((row_id & 1) == 1)

    wait_all(wq_v, wq_sem)
    for j in range(_NPAIR):
        q = jnp.dot(xb, wq_v[:, j * _PAIR:(j + 1) * _PAIR], preferred_element_type=f32)
        qd_ref[j] = jnp.where(own, q, 0.0).astype(bf16)

    scale = _DH ** -0.5

    def pair(j, carry):
        slot = j % 2

        @pl.when(j + 1 < _NPAIR)
        def _():
            start_kv(j + 1, 1 - slot)

        @pl.when(j + 1 == _NPAIR)
        def _():
            start_wo(0)

        wait_all(k_buf.at[slot], kv_sems.at[0, slot])
        s = jnp.dot(qd_ref[j], k_buf[slot], preferred_element_type=f32) * scale
        m = jnp.max(s, axis=1, keepdims=True)
        p = jnp.exp(s - m)
        l = jnp.sum(p, axis=1, keepdims=True)
        wait_all(v_buf.at[slot], kv_sems.at[1, slot])
        o = jax.lax.dot_general(p.astype(bf16), v_buf[slot], (((1,), (1,)), ((), ())),
                                preferred_element_type=f32)
        o = jnp.where(own, o / l, 0.0)
        o_ref[j] = (o[0:1] + o[1:2]).astype(bf16)
        return carry

    jax.lax.fori_loop(0, _NPAIR, pair, 0)

    for g in range(1, len(_WO_GROUPS)):
        start_wo(g)

    acc = jnp.zeros((_ROWS, d), f32)
    for g, group in enumerate(_WO_GROUPS):
        chunks = _wo_chunks(group)
        n, starts0, starts1 = group
        for a in (*starts0, *starts1):
            wait_all(wo_v.at[pl.ds(a, n)], wo_sems.at[g])
        for r0 in chunks:
            j, c = divmod(r0, _PAIR)
            ob = jnp.broadcast_to(o_ref[j, :, c:c + 128], (_ROWS, 128))
            acc += jnp.dot(ob, wo_v[r0:r0 + 128, :], preferred_element_type=f32)

    out_v[...] = (gate * acc[0:1] + b_part).astype(out_v.dtype)
    out_cp.start()
    out_cp.wait()


@jax.jit
def pallas_gated_mix__sliding_block_cached__moe_arch_mod__decode_kernel(
    A_x: jax.Array,
    A_k_cache: jax.Array,
    A_v_cache: jax.Array,
    A_wq: jax.Array,
    A_wo: jax.Array,
    B_x: jax.Array,
    B_w_r: jax.Array,
    B_w_gate: jax.Array,
    B_w_up: jax.Array,
    B_w_down: jax.Array,
    gate_w: jax.Array,
):
    del B_x
    b, sq, d = A_x.shape
    _, hkv, sk, dh = A_k_cache.shape
    w = min(4096, max(256, sk // 4))
    assert (b, sq, hkv, dh) == (1, 1, _HQ, _DH) and w % _KV_C == 0 and (sk - w) % 128 == 0
    assert A_wo.shape[0] == sum(128 * len(_wo_chunks(g)) for g in _WO_GROUPS)
    dt = A_x.dtype
    kt = jnp.swapaxes(A_k_cache, 2, 3).reshape(hkv * dh, sk)
    vt = jnp.swapaxes(A_v_cache, 2, 3).reshape(hkv * dh, sk)

    hbm = pl.BlockSpec(memory_space=pl.ANY)
    vmem = pltpu.VMEM
    dma = pltpu.SemaphoreType.DMA
    return pl.pallas_call(
        functools.partial(_kernel, col0=sk - w),
        in_specs=[hbm] * 10,
        out_specs=hbm,
        out_shape=jax.ShapeDtypeStruct((b, sq, d), dt),
        scratch_shapes=[
            vmem((1, d), dt), vmem(B_w_r.shape, dt), vmem(gate_w.shape, dt),
            vmem(A_wq.shape, dt), vmem(A_wo.shape, dt),
            vmem(B_w_gate.shape, dt), vmem(B_w_up.shape, dt), vmem(B_w_down.shape, dt),
            vmem((2, _PAIR, w), dt), vmem((2, _PAIR, w), dt),
            vmem((_NPAIR, _ROWS, _PAIR), dt), vmem((_NPAIR, 1, _PAIR), dt),
            vmem((1, d), dt),
            dma((4,)), dma((4,)), dma((len(_WO_GROUPS),)), dma((2, 2)),
        ],
        compiler_params=pltpu.CompilerParams(
            vmem_limit_bytes=64 * 1024 * 1024,
            disable_bounds_checks=True, disable_semaphore_checks=True),
    )(A_x, kt, vt, A_wq, A_wo, B_w_r, B_w_gate, B_w_up, B_w_down, gate_w)
```
